```python
import os as _os
_os.environ.setdefault("JAX_PLATFORMS", "cpu")
import jax
import jax.numpy as jnp

def _softmax(x, axis=-1):
    return jax.nn.softmax(x, axis=axis)
def _gelu(x):
    return jax.nn.gelu(x, approximate=True)
def _silu(x):
    return jax.nn.silu(x)
def _sigmoid(x):
    return jax.nn.sigmoid(x)
def _layernorm(x, axis=-1, eps=1e-5):
    m = jnp.mean(x, axis=axis, keepdims=True)
    v = jnp.var(x, axis=axis, keepdims=True)
    return (x - m) / jnp.sqrt(v + eps)
def _scatter_add(tgt, idx, src, axis=0):
    return tgt.at[idx].add(src)
def _segment_sum(src, seg, n):
    return jax.ops.segment_sum(src, seg, n)
class _Rng:
    def __init__(self, key):
        self._k = key
    def _next(self):
        self._k, sub = jax.random.split(self._k)
        return sub
    def normal(self, shape):
        return jax.random.normal(self._next(), shape, dtype=jnp.bfloat16)
    def randint(self, lo, hi, shape):
        return jax.random.randint(self._next(), shape, lo, hi, dtype=jnp.int32)
    def uniform(self, shape, lo=0.0, hi=1.0):
        return jax.random.uniform(self._next(), shape, jnp.bfloat16, lo, hi)
    def permutation(self, n):
        return jax.random.permutation(self._next(), n)


kernel_name = 'concat_heads__gqa_block_cached__mha_block_cached__near_ridge'

def setup_inputs():
    _rng = _Rng(jax.random.key(int.from_bytes(__import__("os").urandom(4), "little")))
    _w = (lambda a: (lambda t: t.astype(jnp.bfloat16) if jnp.issubdtype(t.dtype, jnp.floating) else t)(jnp.asarray(a)))
    def _A_setup():
        B, Sq, D = 8, 224, 512
        Hq, Hkv, Sk, Dh = 32, 32, 512, 128
        assert Hq % Hkv == 0, (Hq, Hkv)
        return {
            "x": _w((lambda *s: _rng.normal(s) * 0.8)(B, Sq, D)),
            "k_cache": _w((lambda *s: _rng.normal(s) * 0.8)(B, Hkv, Sk, Dh)),
            "v_cache": _w((lambda *s: _rng.normal(s) * 0.05)(B, Hkv, Sk, Dh)),
            "wq": _w((lambda *s: _rng.normal(s) * 0.8)(D, Hq * Dh) * (D ** -0.5)),
            "wo": _w((lambda *s: _rng.normal(s) * 0.05)(Hq * Dh, D) * ((Hq * Dh) ** -0.5)),
        }
    _A_in = _A_setup()

    def _B_setup():
        B, Sq, D = 8, 224, 512
        H, Sk, Dh = 32, 512, 128
        return {
            "x": _w((lambda *s: _rng.normal(s) * 0.8)(B, Sq, D)),
            "k_cache": _w((lambda *s: _rng.normal(s) * 0.8)(B, H, Sk, Dh)),
            "v_cache": _w((lambda *s: _rng.normal(s) * 0.05)(B, H, Sk, Dh)),
            "wq": _w((lambda *s: _rng.normal(s) * 0.8)(D, H * Dh) * (D ** -0.5)),
            "wo": _w((lambda *s: _rng.normal(s) * 0.05)(H * Dh, D) * ((H * Dh) ** -0.5)),
        }
    _B_in = _B_setup()

    return {
        "A_x": _A_in["x"],
        "A_k_cache": _A_in["k_cache"],
        "A_v_cache": _A_in["v_cache"],
        "A_wq": _A_in["wq"],
        "A_wo": _A_in["wo"],
        "B_x": _B_in["x"],
        "B_k_cache": _B_in["k_cache"],
        "B_v_cache": _B_in["v_cache"],
        "B_wq": _B_in["wq"],
        "B_wo": _B_in["wo"],
    }

def reference(A_x, A_k_cache, A_v_cache, A_wq, A_wo, B_x, B_k_cache, B_v_cache, B_wq, B_wo):
    def _A_ref(x, k_cache, v_cache, wq, wo):
        B, Sq, D = x.shape
        Hq, Dh = 32, 128
        Hkv = k_cache.shape[1]
        rep = Hq // Hkv
        q = (lambda x, *d: x.transpose(*d))((x @ wq).reshape(B, Sq, Hq, Dh), 0, 2, 1, 3)
        k = jnp.repeat(k_cache, rep, axis=1)
        v = jnp.repeat(v_cache, rep, axis=1)
        scores = jnp.einsum("bhqd,bhkd->bhqk", q, k) * (Dh ** -0.5)
        p = _softmax(scores, axis=-1)
        o = jnp.einsum("bhqk,bhkd->bhqd", p, v)
        return (lambda x, *d: x.transpose(*d))(o, 0, 2, 1, 3).reshape(B, Sq, Hq * Dh) @ wo

    def _B_ref(x, k_cache, v_cache, wq, wo):
        B, Sq, D = x.shape
        H, Dh = 32, 128
        q = (lambda x, *d: x.transpose(*d))((x @ wq).reshape(B, Sq, H, Dh), 0, 2, 1, 3)
        scores = jnp.einsum("bhqd,bhkd->bhqk", q, k_cache) * (Dh ** -0.5)
        p = _softmax(scores, axis=-1)
        o = jnp.einsum("bhqk,bhkd->bhqd", p, v_cache)
        return (lambda x, *d: x.transpose(*d))(o, 0, 2, 1, 3).reshape(B, Sq, H * Dh) @ wo

    a = _A_ref(A_x, A_k_cache, A_v_cache, A_wq, A_wo)
    b = _B_ref(B_x, B_k_cache, B_v_cache, B_wq, B_wo)
    return jnp.concatenate([a, b], axis=-1)
```

```python
import functools
import jax
import jax.numpy as jnp
from jax import lax
import jax.experimental.pallas as pl
import jax.experimental.pallas.tpu as pltpu

B, SQ, D, H, SK, DH = 8, 224, 512, 32, 512, 128
LOG2E = 1.4426950408889634
F32, BF16 = jnp.float32, jnp.bfloat16

def _build(NB=4, G=4, NBUF=3, flags=None, nobounds=False):
    NG = H // G
    NP = B // NB
    PER = NG * NP
    STEPS = 2 * PER

    def kern(ax, ak, av, awq, awo, bx, bk, bv, bwq, bwo, out_hbm,
             x_buf, wq_buf, wo_buf, k_buf, v_buf, acc, o_stage,
             x_sem, wq_sem, wo_sem, k_sem, v_sem, o_sem):
        def coords(t):
            br = t // PER
            r = t % PER
            return br, r // NP, r % NP

        def k_copy(src, hg, bp, slot):
            return pltpu.make_async_copy(src.at[pl.ds(bp * NB, NB), pl.ds(hg * G, G)], k_buf.at[slot], k_sem.at[slot])
        def v_copy(src, hg, bp, slot):
            return pltpu.make_async_copy(src.at[pl.ds(bp * NB, NB), pl.ds(hg * G, G)], v_buf.at[slot], v_sem.at[slot])
        def x_copy(src, br, bp):
            return pltpu.make_async_copy(src.at[pl.ds(bp * NB, NB)], x_buf.at[br, pl.ds(bp * NB, NB)], x_sem.at[br * NP + bp])
        def wq_copy(src, br, hg):
            c = pl.multiple_of(hg * (G * DH), G * DH)
            return pltpu.make_async_copy(src.at[:, pl.ds(c, G * DH)], wq_buf.at[br * NG + hg], wq_sem.at[br * NG + hg])
        def wo_copy(src, br, hg):
            c = pl.multiple_of(hg * (G * DH), G * DH)
            return pltpu.make_async_copy(src.at[pl.ds(c, G * DH)], wo_buf.at[br * NG + hg], wo_sem.at[br * NG + hg])
        def o_copy(br, bp):
            c = pl.multiple_of(br * D, D)
            return pltpu.make_async_copy(o_stage.at[br, pl.ds(bp * NB, NB)], out_hbm.at[pl.ds(bp * NB, NB), :, pl.ds(c, D)], o_sem.at[br * NP + bp])

        def issue(t):
            br, hg, bp = coords(t)
            slot = t % NBUF
            def go(x, k, v, wq, wo):
                @pl.when(hg == 0)
                def _(): x_copy(x, br, bp).start()
                @pl.when(bp == 0)
                def _(): wq_copy(wq, br, hg).start()
                k_copy(k, hg, bp, slot).start()
                v_copy(v, hg, bp, slot).start()
                @pl.when(bp == 0)
                def _(): wo_copy(wo, br, hg).start()
            pl.when(br == 0)(lambda: go(ax, ak, av, awq, awo))
            pl.when(br == 1)(lambda: go(bx, bk, bv, bwq, bwo))

        for t in range(NBUF - 1):
            issue(jnp.int32(t))

        def step(t, carry):
            br, hg, bp = coords(t)
            slot = t % NBUF
            pl.when(t + NBUF - 1 < STEPS)(lambda: issue(t + NBUF - 1))
            @pl.when(hg == 0)
            def _(): x_copy(ax, br, bp).wait()
            @pl.when(bp == 0)
            def _():
                wq_copy(awq, br, hg).wait()
                wo_copy(awo, br, hg).wait()
            k_copy(ak, hg, bp, slot).wait()
            v_copy(av, hg, bp, slot).wait()
            w = br * NG + hg
            units = [(b, h) for b in range(NB) for h in range(G)]
            n = len(units)
            q, p, li, o = {}, {}, {}, {}
            def qproj(i):
                b, h = units[i]
                r = jnp.dot(x_buf[br, bp * NB + b], wq_buf[w, :, h * DH:(h + 1) * DH], preferred_element_type=F32)
                q[i] = (r * (DH ** -0.5 * LOG2E)).astype(BF16)
            def qk(i):
                b, h = units[i]
                s = lax.dot_general(q[i], k_buf[slot, b, h], (((1,), (1,)), ((), ())), preferred_element_type=F32)
                m = jnp.max(s, axis=-1, keepdims=True)
                e = jnp.exp2(s - m)
                l = jnp.sum(e, axis=-1, keepdims=True)
                r = pltpu.reciprocal(l, approx=True)
                li[i] = r * (2.0 - l * r)
                p[i] = e.astype(BF16)
            def pv(i):
                b, h = units[i]
                r = jnp.dot(p[i], v_buf[slot, b, h], preferred_element_type=F32)
                o[i] = (r * li[i]).astype(BF16)
            def outp(b, j):
                oc = jnp.concatenate([o[b * G + h] for h in range(G)], axis=-1)
                r = jnp.dot(oc, wo_buf[w, :, j * 128:(j + 1) * 128], preferred_element_type=F32)
                prev = jnp.where(hg == 0, 0.0, acc[bp * NB + b, :, j * 128:(j + 1) * 128])
                r = r + prev
                acc[bp * NB + b, :, j * 128:(j + 1) * 128] = r
                o_stage[br, bp * NB + b, :, j * 128:(j + 1) * 128] = r.astype(BF16)
            pend = []
            qproj(0)
            if n > 1: qproj(1)
            qk(0)
            for i in range(n):
                if i + 2 < n: qproj(i + 2)
                if i + 1 < n: qk(i + 1)
                if pend: outp(*pend.pop(0))
                pv(i)
                if i % G == G - 1:
                    pend += [(i // G, j) for j in range(4)]
            while pend: outp(*pend.pop(0))
            @pl.when(hg == NG - 1)
            def _(): o_copy(br, bp).start()
            return carry
        lax.fori_loop(0, STEPS, step, 0)
        for br in range(2):
            for bp in range(NP):
                o_copy(br, bp).wait()

    def fn(*args):
        return pl.pallas_call(
            kern,
            in_specs=[pl.BlockSpec(memory_space=pl.ANY)] * 10,
            out_specs=pl.BlockSpec(memory_space=pl.ANY),
            out_shape=jax.ShapeDtypeStruct((B, SQ, 2 * D), BF16),
            scratch_shapes=[
                pltpu.VMEM((2, B, SQ, D), BF16),
                pltpu.VMEM((2 * NG, D, G * DH), BF16),
                pltpu.VMEM((2 * NG, G * DH, D), BF16),
                pltpu.VMEM((NBUF, NB, G, SK, DH), BF16),
                pltpu.VMEM((NBUF, NB, G, SK, DH), BF16),
                pltpu.VMEM((B, SQ, D), F32),
                pltpu.VMEM((2, B, SQ, D), BF16),
                pltpu.SemaphoreType.DMA((2 * NP,)),
                pltpu.SemaphoreType.DMA((2 * NG,)),
                pltpu.SemaphoreType.DMA((2 * NG,)),
                pltpu.SemaphoreType.DMA((NBUF,)),
                pltpu.SemaphoreType.DMA((NBUF,)),
                pltpu.SemaphoreType.DMA((2 * NP,)),
            ],
            compiler_params=pltpu.CompilerParams(
                vmem_limit_bytes=110 * 1024 * 1024, flags=flags, disable_bounds_checks=nobounds),
        )(*args)
    return fn


@jax.jit
def pallas_concat_heads__gqa_block_cached__mha_block_cached__near_ridge_kernel(
    A_x, A_k_cache, A_v_cache, A_wq, A_wo, B_x, B_k_cache, B_v_cache, B_wq, B_wo,
):
    return _build()(A_x, A_k_cache, A_v_cache, A_wq, A_wo, B_x, B_k_cache, B_v_cache, B_wq, B_wo)
```

```python
import math
import jax
import jax.numpy as jnp
from jax import lax
import jax.experimental.pallas as pl
import jax.experimental.pallas.tpu as pltpu

B, SQ, D, H, SK, DH = 8, 224, 512, 32, 512, 128
LOG2E = 1.4426950408889634
F32, BF16 = jnp.float32, jnp.bfloat16
NC = SQ // 16


class Lin:
    def __init__(self, terms=(), scale=1.0, key=None):
        self.terms, self.scale, self.key = tuple(terms), scale, key


def lin(*terms, scale=1.0):
    terms = [(c, n) for c, n in terms if abs(c) > 1e-12]
    if len(terms) == 1 and terms[0][0] == 1 and scale == 1.0:
        return terms[0][1]
    return Lin(terms, scale)


class Strassen:
    m, R = 2, 7
    T = {"a": [((1, 0, 0), (1, 1, 1)), ((1, 1, 0), (1, 1, 1)), ((1, 0, 0),), ((1, 1, 1),),
               ((1, 0, 0), (1, 0, 1)), ((1, 1, 0), (-1, 0, 0)), ((1, 0, 1), (-1, 1, 1))],
         "b": [((1, 0, 0), (1, 1, 1)), ((1, 0, 0),), ((1, 0, 1), (-1, 1, 1)), ((1, 1, 0), (-1, 0, 0)),
               ((1, 1, 1),), ((1, 0, 0), (1, 0, 1)), ((1, 1, 0), (1, 1, 1))],
         "c": [((1, 0, 0), (1, 1, 1)), ((1, 1, 0), (-1, 1, 1)), ((1, 0, 1), (1, 1, 1)), ((1, 0, 0), (1, 1, 0)),
               ((1, 0, 1), (-1, 0, 0)), ((1, 1, 1),), ((1, 0, 0),)]}

    def __init__(self, order):
        self.order = order

    def fwd(self, side, get):
        return [lin(*[(c, get(r, s)) for c, r, s in self.T[side][p]]) for p in self.order]

    def bwd(self, side, prods):
        out = {}
        for p, node in zip(self.order, prods):
            for c, r, s in self.T[side][p]:
                out.setdefault((r, s), []).append((c, node))
        return {k: lin(*v) for k, v in out.items()}


class HK:
    def __init__(self, m, theta=None, reverse=False):
        self.m, self.R = m, (3 * m * m + m) // 2
        self.th = theta or [1.0 / math.tan(math.pi * (i + 1) / (m + 1)) for i in range(m)]
        self.pairs = [(i, j) for j in range(m) for i in range(j)]

    def fwd(self, side, get):
        m, th = self.m, self.th
        out = []
        if side == "a":
            X = [get(i, 0) for i in range(m)]
            Y = [lin((1, get(i, 1)), (th[i], X[i])) for i in range(m)]
            for i in range(m): out += [X[i], Y[i]]
            for i, j in self.pairs:
                s = lin((1, Y[i]), (-1, Y[j]), scale=1.0 / (th[j] - th[i]))
                out += [s, lin((1, X[i]), (1, s)), lin((1, X[j]), (1, s))]
        elif side == "b":
            G = [get(1, j) for j in range(m)]
            Fm = [lin((1, get(0, j)), (-th[j], G[j])) for j in range(m)]
            for i in range(m): out += [Fm[i], G[i]]
            for i, j in self.pairs:
                d = th[j] - th[i]
                s = lin((1, Fm[j]), (-1, Fm[i]))
                out += [s, lin((1, s), (d, G[j])), lin((-d, G[i]), (-1, s))]
        else:
            for i in range(m):
                out += [lin(*[(1, get(i, j)) for j in range(m)]), lin(*[(1, get(j, i)) for j in range(m)])]
            for i, j in self.pairs:
                out += [lin((1, get(j, i)), (-1, get(i, j))), get(i, j), get(j, i)]
        return out

    def bwd(self, side, prods):
        m, th = self.m, self.th
        Dp, Ep = prods[0:2 * m:2], prods[1:2 * m:2]
        trip = {pr: prods[2 * m + 3 * n: 2 * m + 3 * n + 3] for n, pr in enumerate(self.pairs)}
        out = {}
        if side == "c":
            for i in range(m): out[i, i] = lin((1, Dp[i]), (1, Ep[i]))
            for (i, j), (s, tij, tji) in trip.items():
                out[i, j] = lin((1, Dp[i]), (1, Ep[j]), (-1, s), (1, tij))
                out[j, i] = lin((1, Dp[j]), (1, Ep[i]), (1, s), (1, tji))
        else:
            xs = [[(1, Dp[i])] for i in range(m)]
            ys = [[(1, Ep[i])] for i in range(m)]
            for (i, j), (s, tij, tji) in trip.items():
                z = lin((1, s), (1, tij), (1, tji), scale=1.0 / (th[j] - th[i]))
                xs[i].append((1, tij)); xs[j].append((1, tji))
                ys[i].append((1, z)); ys[j].append((-1, z))
            for i in range(m):
                y = lin(*ys[i])
                out[i, 1] = y
                out[i, 0] = lin(*xs[i], (th[i], y))
        return out


def nest_fwd(s1, s2, side):
    dims = lambda s: {"a": (s.m, 2), "b": (2, s.m), "c": (s.m, s.m)}[side]
    r2, c2 = dims(s2)
    cache = {}
    def get(r, c):
        if (r, c) not in cache: cache[r, c] = Lin(key=(r, c))
        return cache[r, c]
    lvl1 = {(r, c): s1.fwd(side, lambda i, k, r=r, c=c: get(i * r2 + r, k * c2 + c))
            for r in range(r2) for c in range(c2)}
    out = []
    for p in range(s1.R):
        out += s2.fwd(side, lambda r, c, p=p: lvl1[r, c][p])
    return out


def nest_bwd(s1, s2, side):
    dims = lambda s: {"a": (s.m, 2), "c": (s.m, s.m)}[side]
    r2, c2 = dims(s2)
    prods = [Lin(key=(p,)) for p in range(s1.R * s2.R)]
    inner = [s2.bwd(side, prods[p * s2.R:(p + 1) * s2.R]) for p in range(s1.R)]
    out = {}
    for r in range(r2):
        for c in range(c2):
            for (i, k), node in s1.bwd(side, [inner[p][r, c] for p in range(s1.R)]).items():
                out[i * r2 + r, k * c2 + c] = node
    return out


def leaves(node):
    if not node.terms: return [node.key]
    return list(dict.fromkeys(k for _, ch in node.terms for k in leaves(ch)))


def evaluate(node, leaf, cache):
    if id(node) not in cache:
        if not node.terms:
            cache[id(node)] = leaf(*node.key)
        else:
            acc = None
            for c, ch in sorted(node.terms, key=lambda t: t[0] == -1):
                v = evaluate(ch, leaf, cache).astype(F32)
                if acc is None: acc = v if c == 1 else v * c
                elif c == 1: acc = acc + v
                elif c == -1: acc = acc - v
                else: acc = acc + v * c
            cache[id(node)] = acc if node.scale == 1.0 else acc * node.scale
    return cache[id(node)]


def run(gen):
    for _ in gen: pass


def scheme(name):
    if name[0] == '_': return Strassen(tuple(int(c) for c in name[1:]))
    return {"Sq": Strassen((2, 4, 5, 6, 0, 1, 3)), "So": Strassen((6, 4, 3, 5, 2, 0, 1)), "Si": Strassen((4, 6, 5, 1, 0, 2, 3)), "H2": HK(2), "H4": HK(4)}[name]


def plan_push(outs, groups):
    topo, seen, parents, prods = [], set(), {}, {}
    def visit(n):
        if id(n) in seen: return
        seen.add(id(n))
        for _, ch in n.terms:
            visit(ch); parents.setdefault(id(ch), []).append(n)
        if n.terms: topo.append(n)
        else: prods[n.key[0]] = n
    for n in outs.values(): visit(n)
    have, where, plan = set(), {}, []
    for members in groups:
        fresh = [prods[p] for p in members]
        have.update(id(n) for n in fresh)
        for n in topo:
            if id(n) not in have and all(id(ch) in have for _, ch in n.terms):
                have.add(id(n)); fresh.append(n)
        park = [n for n in fresh if any(id(q) not in have for q in parents.get(id(n), ()))]
        now = {id(n) for n in fresh}
        plan.append((fresh, dict(where), len(where), park, [(k, n) for k, n in outs.items() if id(n) in now]))
        for n in park: where[id(n)] = len(where)
    return plan, len(where)


def build(QS="Sq.Sq", OS="So.Si", LAG=11, LAGO=11, LS=11, LX=9, PC=7, LO=14, newton=True, WQ=2, WO=1, presum=True,
          flags="XLA_TPU_RESCHEDULE_DMA_DONES", nobounds=True, only="qao", nodma=False, natt=32):
    if isinstance(flags, str): flags = {f: True for f in flags.split("+")}
    q1, q2 = [scheme(n) for n in QS.split(".")]
    o1, o2 = [scheme(n) for n in OS.split(".")]
    G, R = 8, 49
    NG = H // G
    STEPS = 4 * NG

    x_roots, wq_roots, q_outs = nest_fwd(q1, q2, "a"), nest_fwd(q1, q2, "b"), nest_bwd(q1, q2, "c")
    o_roots, wo_roots, y_outs = nest_fwd(o1, o2, "c"), nest_fwd(o1, o2, "b"), nest_bwd(o1, o2, "a")
    groups = [list(range(p, min(p + 2, R))) for p in range(0, R, 2)]
    y_plan, parked = plan_push(y_outs, groups)

    top = [0]
    def region(n):
        top[0] += n
        return top[0] - n
    S0, L0, O0, W0, M0, Y0 = region(8), region(1), region(32), region(2 * R), region(parked), region(16)
    pre = {}
    def collect(n):
        if n.terms and all(not ch.terms for _, ch in n.terms):
            (i0, j0), (i1, j1) = [ch.key for _, ch in n.terms]
            if (i0 // 2, j0 // 2) != (i1 // 2, j1 // 2) and id(n) not in pre: pre[id(n)] = (n, region(2))
        for _, ch in n.terms: collect(ch)
    if presum:
        for r in o_roots: collect(r)
    def home(n):
        return pre[id(n)][1] if id(n) in pre else None if n.terms else O0 + 8 * n.key[0] + 2 * n.key[1]
    def sources(n):
        return [n] if home(n) is not None else [m for _, ch in n.terms for m in sources(ch)]
    last_q = lambda i, j: max(p for p, in leaves(q_outs[i, j]))
    first_o = lambda i, j: min(p for p in range(R) if (i, j) in leaves(o_roots[p]))
    border = sorted(range(4), key=lambda i: min(last_q(i, j) for j in range(4)))
    units = [(i, 2 * j + u) for i in border
             for j in sorted(range(4), key=lambda j: last_q(i, j) if i != border[-1] else first_o(i, j)) for u in range(2)][:natt]
    xorder = list(dict.fromkeys(i for r in x_roots for i, _ in leaves(r)))
    worder = list(dict.fromkeys(j for r in wq_roots for _, j in leaves(r)))

    def kern(ax, ak, av, awq, awo, bx, bk, bv, bwq, bwo, out_hbm,
             ar, x_buf, wq_buf, wo_buf, k_buf, v_buf, y_buf, sem):
        class Nop:
            def start(self): pass
            def wait(self): pass
        mk = (lambda *a: Nop()) if nodma else pltpu.make_async_copy
        batch = lambda t, i: 4 * ((t >> 2) & 1) + i
        def k_copy(src, t, i, j):
            return mk(src.at[batch(t, i), pl.ds((t & 3) * G + 2 * j, 2)], k_buf.at[i, pl.ds(2 * j, 2)], sem.at[4 * i + j])
        def v_copy(src, t, i, j):
            return mk(src.at[batch(t, i), pl.ds((t & 3) * G + 2 * j, 2)], v_buf.at[i, pl.ds(2 * j, 2)], sem.at[16 + 4 * i + j])
        def x_copy(src, t, i):
            return mk(src.at[batch(t, i)], x_buf[i], sem.at[32 + i])
        def wq_copy(src, t, j):
            c = pl.multiple_of(((t & 3) * 4 + j) * 256, 256)
            return mk(src.at[:, pl.ds(c, 256)], wq_buf[j].at[t & 3], sem.at[36 + j])
        def wo_copy(src, t):
            c = pl.multiple_of((t & 3) * (G * DH), G * DH)
            return mk(src.at[pl.ds(c, G * DH)], wo_buf.at[t & 3], sem.at[40])
        def y_copy(t, i):
            c = pl.multiple_of((t >> 3) * D, D)
            return mk(y_buf.at[t >> 2, i], out_hbm.at[batch(t, i), :, pl.ds(c, D)], sem.at[41 + 4 * (t >> 2) + i])
        def start(copy, a_src, b_src, t, mask, *args):
            pl.when((t & (24 | mask)) == 0)(lambda: copy(a_src, t, *args).start())
            pl.when((t & (24 | mask)) == 8)(lambda: copy(b_src, t, *args).start())

        T = lambda i: slice(i * 128, (i + 1) * 128)

        class Block:
            def __init__(self, zero):
                self.zero = zero
                self.events, self.now = {}, 0
                self.pending = {}
                self.tie = None
            def at(self, t, fn): self.events.setdefault(max(t, self.now), []).append(fn)
            def tick(self):
                for fn in self.events.pop(self.now, []): fn()
                self.now += 1
            def drain(self):
                while self.events: self.tick()
            def put(self, t0, blk, row, val):
                nb, n = val.shape[0], val.shape[1] // 16
                for b in range(blk, blk + nb): self.pending[b] = self.pending.get(b, 0) + n
                def one(c):
                    ar[pl.ds(blk, nb), pl.ds(row + 16 * c, 16), :] = val[:, 16 * c:16 * c + 16]
                    for b in range(blk, blk + nb): self.pending[b] -= 1
                for c in range(n): self.at(t0 + c, lambda c=c: one(c))
            def get(self, blk):
                assert not self.pending.get(blk, 0)
                return ar[blk]
            def paced(self, blk, row=0, rows=SQ, step=16):
                out = []
                for r in range(row, row + rows, step):
                    self.tick()
                    v = ar[self.zero + blk, pl.ds(r, step), :]
                    if self.tie is not None and step == 16:
                        v = jnp.where(self.zero == 0, v, self.tie())
                        self.tie = None
                    out.append(v)
                return jnp.concatenate(out, 0)

            def products(self, lhs, rhs, sink, wmode):
                wcache = {}
                for g, members in enumerate(groups):
                    n = len(members)
                    ws = [rhs(p, wcache) for p in members]
                    vals = lhs(members, 32 // n)
                    t0 = self.now - NC * n // 2
                    if wmode == 1:
                        for k in [k for k, v in wcache.items() if v.dtype == BF16]: del wcache[k]
                    if wmode == 2: wcache.clear()
                    for r0 in range(0, SQ, SQ * n // 2):
                        r1 = r0 + SQ * n // 2
                        sink(g, t0, r0, [jnp.dot(v[r0:r1].astype(BF16), w, preferred_element_type=F32) for v, w in zip(vals, ws)])
                    yield

            def qproj(self, t):
                seen = set()
                def lhs(members, step):
                    for i in dict.fromkeys(i for p in members for i, _ in leaves(x_roots[p])):
                        if ("x", i) not in seen:
                            seen.add(("x", i))
                            pl.when((t & 3) == 0)(x_copy(ax, t, i).wait)
                    for p in range(members[-1] + 1, min(members[-1] + 3, R)): arrive(p)
                    cache = {}
                    vals = [evaluate(x_roots[p], lambda i, k: x_buf[i][:, T(k)], cache) for p in members]
                    vals[0] = jnp.where(self.zero == 0, vals[0].astype(F32), self.paced(S0, step=step))
                    return vals
                def arrive(p):
                    for j in dict.fromkeys(j for _, j in leaves(wq_roots[p])):
                        if j not in seen:
                            seen.add(j)
                            pl.when((t & 4) == 0)(wq_copy(awq, t, j).wait)
                arrive(0); arrive(1)
                def rhs(p, wcache):
                    return evaluate(wq_roots[p], lambda k, j: wq_buf[j][t & 3, T(k), :], wcache).astype(BF16)
                def sink(g, t0, r0, res):
                    self.put(t0 + LAG, W0 + 4 * g, r0, jnp.stack([r[:, T(u)] for r in res for u in range(2)]))
                return self.products(lhs, rhs, sink, WQ)

            def oproj(self, t):
                left = {i: 4 * SQ // 16 for i in range(4)}
                def lhs(members, step):
                    cache = {}
                    for n in [n for p in members for n in sources(o_roots[p])]:
                        if id(n) not in cache:
                            assert not self.pending.get(home(n), 0)
                            cache[id(n)] = jnp.concatenate([self.get(home(n)) if cache else self.paced(home(n), step=step),
                                                            self.get(home(n) + 1)], 1)
                    return [evaluate(o_roots[p], None, cache) for p in members]
                rhs = lambda p, wcache: evaluate(wo_roots[p], lambda k, j: wo_buf[t & 3, pl.ds(256 * j, 256), T(k)], wcache).astype(BF16)
                def sink(g, t0, r0, res):
                    fresh, where, slot, park, finished = y_plan[g]
                    rows = pl.ds(r0, res[0].shape[0])
                    regs = {id(n): r for n, r in zip(fresh, res)}
                    for n in fresh[len(res):]:
                        for _, ch in n.terms:
                            if id(ch) not in regs:
                                while self.pending[M0 + where[id(ch)]]: self.tick()
                                regs[id(ch)] = ar[M0 + where[id(ch)], rows, :]
                        evaluate(n, None, regs)
                    if park: self.put(t0 + LAGO, M0 + slot, r0, jnp.stack([regs[id(n)] for n in park]))
                    for (i, k), n in finished:
                        val = regs[id(n)] + jnp.where((t & 3) == 0, 0.0, ar[Y0 + 4 * i + k, rows, :])
                        self.put(t0 + LAGO, Y0 + 4 * i + k, r0, val[None])
                        def one(c, i=i, k=k, val=val.astype(BF16)):
                            idx = (t >> 2, i, pl.ds(r0 + 16 * c, 16), T(k))
                            y_buf[idx] = val[16 * c:16 * c + 16]
                            self.tie = lambda: y_buf[(self.zero,) + idx[1:]].astype(F32)
                            left[i] -= 1
                            if not left[i]: pl.when((t & 3) == 3)(y_copy(t, i).start)
                        for c in range(val.shape[0] // 16): self.at(t0 + LAGO + c, lambda c=c, one=one: one(c))
                return self.products(lhs, rhs, sink, WO)

            def attention(self, t, follow):
                def qk(n):
                    i, h = units[n]
                    if n % 2 == 0: k_copy(ak, t, i, h // 2).wait()
                    root = q_outs[i, h // 2]
                    first = leaves(root)[0][0]
                    assert not self.pending.get(W0 + 2 * first + h % 2, 0)
                    lead = self.paced(W0 + 2 * first + h % 2)
                    q = evaluate(root, lambda p: lead if p == first else self.get(W0 + 2 * p + h % 2), {})
                    q = (q * (DH ** -0.5 * LOG2E)).astype(BF16)
                    sc = lax.dot_general(q, k_buf[i, h], (((1,), (1,)), ((), ())), preferred_element_type=F32)
                    self.put(self.now - NC + LS, S0 + (n % 2) * 4, 0, jnp.stack([sc[:, T(j)] for j in range(4)]))
                    if n % 2 == 1: start(k_copy, ak, bk, t + 1, 0, i, h // 2)
                def gate(n, t0):
                    blk, got = S0 + (n % 2) * 4, []
                    def one(c):
                        assert self.pending[blk] < NC - c
                        got.append(ar[self.zero + blk, pl.ds(16 * c, 16), :])
                    for c in range(NC): self.at(t0 + c - LX, lambda c=c: one(c))
                    return got
                def pv(n, got):
                    i, h = units[n]
                    if n % 2 == 0: v_copy(av, t, i, h // 2).wait()
                    blk = S0 + (n % 2) * 4
                    parts = []
                    for c0 in range(0, NC, PC):
                        rows = pl.ds(16 * c0, 16 * PC)
                        sc = [jnp.concatenate(got[c0:c0 + PC], 0)] + [ar[blk + j, rows, :] for j in range(1, 4)]
                        m = jnp.max(jnp.maximum(jnp.maximum(sc[3], sc[1]), jnp.maximum(sc[2], sc[0])), axis=-1, keepdims=True)
                        sc = ar[pl.ds(blk, 4), rows, :]
                        e = jnp.exp2(jnp.concatenate([sc[j] - m for j in range(4)], 1))
                        self.put(self.now, L0, 16 * c0, ((e[:, T(0)] + e[:, T(1)]) + (e[:, T(2)] + e[:, T(3)]))[None])
                        lead = jnp.where(self.zero == 0, e[:, T(0)], self.paced(blk, 16 * c0, 16 * PC))
                        parts.append(jnp.concatenate([lead, e[:, 128:]], 1))
                    o = jnp.dot(jnp.concatenate(parts, 0).astype(BF16), v_buf[i, h], preferred_element_type=F32)
                    l = jnp.sum(self.get(L0), axis=-1, keepdims=True)
                    r = pltpu.reciprocal(l, approx=True)
                    if newton: r = r * (2.0 - l * r)
                    o = o * r
                    self.put(self.now - NC + LO, O0 + 8 * i + h, 0, o[None])
                    for node, dst in pre.values():
                        keys = [(a, 2 * b + h % 2) for a, b in leaves(node)]
                        if (i, h) in keys and all(k in units[:n + 1] for k in keys):
                            val = evaluate(node, lambda a, b: o if (a, b) == (i, h // 2) else self.get(O0 + 8 * a + 2 * b + h % 2), {})
                            self.put(self.now - NC + LO, dst + h % 2, 0, val[None])
                    if n % 2 == 1: start(v_copy, av, bv, t + 1, 0, i, h // 2)
                qk(0)
                for n in range(len(units)):
                    got = gate(n, self.now + NC)
                    if n + 1 < len(units): qk(n + 1)
                    else: follow()
                    pv(n, got)

        for i, j in zip(xorder, worder):
            wq_copy(awq, 0, j).start(); x_copy(ax, 0, i).start()
        for i, h in units[::2]:
            k_copy(ak, 0, i, h // 2).start(); v_copy(av, 0, i, h // 2).start()
        wo_copy(awo, 0).start()

        def step(t, carry):
            blk = Block(t >> 8)
            if "q" in only: run(blk.qproj(t))
            def refill():
                for i, j in zip(xorder, worder):
                    start(wq_copy, awq, bwq, t + 1, 4, j); start(x_copy, ax, bx, t + 1, 3, i)
            blk.at(blk.now + NC, refill)
            op = blk.oproj(t)
            def follow():
                pl.when((t & 4) == 0)(wo_copy(awo, t).wait)
                start(wo_copy, awo, bwo, t + 1, 4)
                next(op)
            if "a" in only: blk.attention(t, follow)
            if "o" in only: run(op)
            blk.drain()
            return t >> 8
        z = lax.fori_loop(0, STEPS, step, 0)
        for t in range(3, STEPS, 4):
            for i in range(4): y_copy(t, i).wait()
        if nodma or only != "qao":
            y_buf[0, 0, :, :128] = ar[z].astype(BF16)
            pltpu.sync_copy(y_buf.at[0, 0], out_hbm.at[0, :, pl.ds(0, D)])

    def fn(*args):
        return pl.pallas_call(
            kern,
            in_specs=[pl.BlockSpec(memory_space=pl.ANY)] * 10,
            out_specs=pl.BlockSpec(memory_space=pl.ANY),
            out_shape=jax.ShapeDtypeStruct((B, SQ, 2 * D), BF16),
            scratch_shapes=[
                pltpu.VMEM((top[0], SQ, 128), F32),
                [pltpu.VMEM((SQ, D), BF16)] * 4,
                [pltpu.VMEM((NG, D, 256), BF16)] * 4,
                pltpu.VMEM((NG, G * DH, D), BF16),
                pltpu.VMEM((4, G, SK, DH), BF16),
                pltpu.VMEM((4, G, SK, DH), BF16),
                pltpu.VMEM((4, 4, SQ, D), BF16),
                pltpu.SemaphoreType.DMA((57,)),
            ],
            compiler_params=pltpu.CompilerParams(
                vmem_limit_bytes=100 * 1024 * 1024, flags=flags, disable_bounds_checks=nobounds),
        )(*args)
    return fn


@jax.jit
def pallas_concat_heads__gqa_block_cached__mha_block_cached__near_ridge_kernel(
    A_x, A_k_cache, A_v_cache, A_wq, A_wo, B_x, B_k_cache, B_v_cache, B_wq, B_wo,
):
    return build(LS=10, LO=13)(A_x, A_k_cache, A_v_cache, A_wq, A_wo, B_x, B_k_cache, B_v_cache, B_wq, B_wo)
```

```python
import functools

import jax
import jax.numpy as jnp
from jax import lax
import jax.experimental.pallas as pl
import jax.experimental.pallas.tpu as pltpu

B, SQ, D, SK, DH = 8, 224, 512, 512, 128
HQ = SQ // 2
NC = SQ // 16
G = 8
STEPS = 16
Q_SCALE = DH ** -0.5 * 1.4426950408889634
X_BLOCKS = 92
F32, BF16 = jnp.float32, jnp.bfloat16

A_SIDE = (((1, 0, 0), (1, 1, 1)), ((1, 1, 0), (1, 1, 1)), ((1, 0, 0),), ((1, 1, 1),),
          ((1, 0, 0), (1, 0, 1)), ((1, 1, 0), (-1, 0, 0)), ((1, 0, 1), (-1, 1, 1)))
B_SIDE = (((1, 0, 0), (1, 1, 1)), ((1, 0, 0),), ((1, 0, 1), (-1, 1, 1)), ((1, 1, 0), (-1, 0, 0)),
          ((1, 1, 1),), ((1, 0, 0), (1, 0, 1)), ((1, 1, 0), (1, 1, 1)))
C_SIDE = (((1, 0, 0), (1, 1, 1)), ((1, 1, 0), (-1, 1, 1)), ((1, 0, 1), (1, 1, 1)), ((1, 0, 0), (1, 1, 0)),
          ((1, 0, 1), (-1, 0, 0)), ((1, 1, 1),), ((1, 0, 0),))
HK_OUT = {(0, 0): ((0, 1), ()), (1, 1): ((2, 3), ()), (2, 2): ((4, 5), ()), (3, 3): ((6, 7), ()),
          (0, 1): ((1, 2, 8), (20,)), (1, 0): ((0, 3, 9, 20), ()), (0, 2): ((0, 4, 10, 21), ()),
          (2, 0): ((1, 5, 11), (21,)), (1, 2): ((2, 5, 12), (22,)), (2, 1): ((3, 4, 13, 22), ()),
          (1, 3): ((3, 6, 15, 23), ()), (3, 1): ((2, 7, 14), (23,)), (2, 3): ((5, 7, 17), (24,)),
          (3, 2): ((4, 6, 16, 24), ()), (0, 3): ((1, 2, 8, 14, 18), (20, 0, 25)),
          (3, 0): ((0, 3, 9, 20, 15, 19, 25), (1,))}

TUNING = dict(
    q_outer="4210356",
    q_inner=("yfbucioxhdvrlapjztgqskwenm", "buciyflavxhodpjzwenmgqsktr"),
    q_absorb=(12, 6),
    o_order="44464541060451550010565420666460303663610525535062652624141601033331434052021311212322421535323412",
    pairs="3b19208a75fd64ec",
    sums="22222122221222122222221222322223",
    x_jobs="00111112112222111111112011111111",
    x_lag="22122222212222122422236202322222",
    q_tail="00662010606064666666667666666661",
    s_lag="aba9aabababaaa9aaaaaaabaaaaaaaaa",
    o_lag="cccccbccebcccceececdcccdcccccced",
    l_lag="31111110312111121122121321112101",
    max_lead="9999999999999a99999a9999aa999999",
    q_lag=10, y_lag=11, wo_wait=31,
)


class Sum:
    def __init__(self, terms=(), key=None):
        self.terms, self.key = tuple(terms), key


def signed(terms):
    return terms[0][1] if len(terms) == 1 else Sum(terms)


def add(a, b):
    return Sum([(1, a), (1, b)])


def sub(a, b):
    return Sum([(1, a), (-1, b)])


def leaves(node):
    if not node.terms:
        return [node.key]
    return list(dict.fromkeys(k for _, ch in node.terms for k in leaves(ch)))


def accumulate(acc, terms):
    for s, v in sorted(terms, key=lambda t: -t[0]):
        acc = (v if s > 0 else -v) if acc is None else acc + v if s > 0 else acc - v
    return acc


def evaluate(node, leaf, cache):
    if node not in cache:
        if node.terms:
            cache[node] = accumulate(None, [(s, widened(ch, leaf, cache)) for s, ch in node.terms])
        else:
            cache[node] = leaf(*node.key)
    return cache[node]


def widened(node, leaf, cache):
    if (node, F32) not in cache:
        cache[node, F32] = evaluate(node, leaf, cache).astype(F32)
    return cache[node, F32]


def hk_lhs(x, y):
    z, n2, d = [add(x[i], y[i]) for i in range(4)], Sum([(-1, x[2])]), sub(x[1], x[3])
    return [z[0], y[0], x[1], y[1], n2, z[2], z[3], y[3],
            sub(x[0], x[1]), sub(z[1], z[0]), sub(x[0], x[2]), sub(y[2], y[0]), sub(z[1], z[2]), sub(y[2], y[1]),
            d, sub(z[3], z[1]), sub(x[2], x[3]), sub(y[3], y[2]), sub(x[0], d), sub(add(y[0], y[3]), y[1]),
            sub(x[1], z[0]), sub(n2, y[0]), sub(z[2], y[1]), sub(x[1], z[3]), sub(n2, y[3]),
            sub(sub(x[3], x[1]), y[0])]


def hk_rhs(f, g):
    h, d = [sub(g[j], f[j]) for j in range(4)], sub(g[1], g[3])
    return [f[0], h[0], f[1], g[1], h[2], g[2], f[3], h[3],
            sub(h[0], h[1]), sub(g[0], g[1]), sub(f[2], f[0]), sub(g[0], g[2]), sub(f[2], f[1]), sub(h[1], h[2]),
            sub(h[1], h[3]), d, sub(f[3], f[2]), sub(g[2], g[3]), sub(add(f[0], f[3]), f[1]), sub(g[0], d),
            sub(g[1], h[0]), sub(f[0], g[2]), add(f[1], h[2]), sub(g[1], h[3]), sub(f[3], g[2]), sub(f[0], d)]


def query_plan(order, budget):
    x = {(b, i, k): Sum(key=(b, i, k)) for b in range(4) for i in range(2) for k in range(4)}
    w = {(k, h): Sum(key=(k, h)) for k in range(4) for h in range(G)}
    lhs = [hk_lhs(*[[signed([(s, x[b, i, 2 * k + c]) for s, i, k in A_SIDE[p]]) for b in range(4)]
                    for c in range(2)]) for p in range(7)]
    rhs = [hk_rhs(*[[signed([(s, w[2 * k + c, 4 * j + h]) for s, k, j in B_SIDE[p]]) for h in range(4)]
                    for c in range(2)]) for p in range(7)]
    pos = {pq: n for n, pq in enumerate(order)}
    outs = {}
    for p in range(7):
        for s, i, j in C_SIDE[p]:
            for (b, h), both in HK_OUT.items():
                for sign, qs in zip((1, -1), both):
                    for q in qs:
                        outs.setdefault((b, i, 4 * j + h), {})[pos[p, q]] = s * sign
    absorbed, left = {}, 0
    for n in range(len(order)):
        if n % 4 == 2 and n > 2:
            left = budget[len(B_SIDE[order[min(n + 8, len(order) - 1)][0]]) - 1]
        users = [o for o in outs.values() if n in o]
        for m in range(n - 1, -1, -1):
            ratios = [o.get(m, 0) * o[n] for o in users]
            if left and ratios[0] and all(r == ratios[0] for r in ratios):
                left -= 1
                absorbed.setdefault(n, []).append((ratios[0], m))
                for o in users:
                    del o[m]
    return lhs, [rhs[p][q] for p, q in order], outs, absorbed


def strassen_operands(side, order):
    leaf = {(r, c): Sum(key=(r, c)) for r in range(4) for c in range(4)}
    outer = {(p, r, c): signed([(s, leaf[2 * i + r, 2 * k + c]) for s, i, k in side[p]])
             for p in range(7) for r in range(2) for c in range(2)}
    return [signed([(s, outer[p, r, c]) for s, r, c in side[q]]) for p, q in order]


def fold_plan(order):
    seen, plan = {}, []

    def advance(key, terms, r, c):
        before = seen.get(key, 0)
        seen[key] = before + len(terms)
        return key, terms, before > 0, seen[key] == sum((i, k) == (r, c) for side in A_SIDE for _, i, k in side)

    for first in range(0, len(order), 2):
        inner, outer = {}, {}
        for n, (p, q) in enumerate(order[first:first + 2]):
            for s, r, c in A_SIDE[q]:
                inner.setdefault((p, r, c), []).append((s, n))
        inner = [advance(key, terms, *key[1:]) for key, terms in inner.items()]
        for (p, r, c), _, _, complete in inner:
            for s, i, k in A_SIDE[p] if complete else ():
                outer.setdefault((2 * i + r, 2 * k + c), []).append((s, (p, r, c)))
        plan.append((inner, [advance(key, terms, key[0] // 2, key[1] // 2) for key, terms in outer.items()]))
    return plan


def lanes(i):
    return pl.ds(i * 128, 128)


def column(v, j):
    return v[:, j * 128:(j + 1) * 128]


class Timeline:
    def __init__(self, zero, current):
        self.zero, self.current, self.index = zero, current, {}
        self.events, self.reads, self.pending, self.ties = {}, {}, {}, {}
        self.now = self.phase = 0

    def at(self, t, fn):
        self.events.setdefault(max(t, self.now), []).append(fn)

    def tick(self):
        for fn in self.events.pop(self.now, []) + self.reads.pop(self.now, []):
            fn()
        self.now += 1

    def put(self, t0, ref, blk, row, vals, by=1 << 30):
        val, n = jnp.stack(vals), vals[0].shape[0] // 16
        keys = [(id(ref), b) for b in range(blk, blk + len(vals))]
        for key in keys:
            self.pending[key] = self.pending.get(key, 0) + n

        def store(c0, c1):
            ref[pl.ds(blk, len(vals)), pl.ds(row + 16 * c0, 16 * (c1 - c0)), :] = val[:, 16 * c0:16 * c1]
            for key in keys:
                self.pending[key] -= c1 - c0

        self.spread(t0, n, store, by)

    def spread(self, t0, n, fn, by=1 << 30):
        due = [max(min(t0 + c, by), self.now) for c in range(n)]
        c0 = 0
        for c in range(n):
            if c + 1 == n or (due[c] + self.phase) // 2 != (due[c + 1] + self.phase) // 2:
                self.at(due[c], lambda span=(c0, c + 1): fn(*span))
                c0 = c + 1

    def get(self, ref, blk):
        assert self.pending[id(ref), blk] == 0
        return ref[blk]

    def ordered(self, blk):
        if blk not in self.index:
            self.index[blk] = self.zero + blk
        return self.index[blk]

    def marker(self, rows=8):
        return self.current[self.ordered(self.current.shape[0] - 1), pl.ds(0, rows), :]

    def paced(self, val, rows=None, step=16):
        out, done = [], 0
        for r in range(0, rows or val.shape[0], step):
            self.tick()
            if self.now % 2 == self.phase:
                w = self.marker()
                for tie in self.ties.values():
                    w = jnp.where(self.zero == 0, w, pltpu.bitcast(tie(), F32))
                self.ties = {}
                out += ([val[done:r]] if r > done else []) + [jnp.where(self.zero == 0, val[r:r + 8], w)]
                done = r + 8
        return jnp.concatenate(out + ([val[done:]] if done < val.shape[0] else []), 0)


def build():
    knob = lambda name, n: int(TUNING[name][n], 16)
    q_order = [(int(p), ord(c) - ord("a")) for n, p in enumerate(TUNING["q_outer"]) for c in TUNING["q_inner"][n % 2]]
    o_order = [(int(p), int(q)) for p, q in zip(TUNING["o_order"][::2], TUNING["o_order"][1::2])]
    x_roots, wq_roots, q_outs, absorbed = query_plan(q_order, TUNING["q_absorb"])
    o_roots, wo_roots = strassen_operands(C_SIDE, o_order), strassen_operands(B_SIDE, o_order)
    y_plan = fold_plan(o_order)
    wq_parts = lambda roots: list(dict.fromkeys((k // 2, h // 4) for n in roots for k, h in leaves(n)))
    wo_parts = lambda roots: list(dict.fromkeys((k // 2, j // 2) for n in roots for k, j in leaves(n)))
    pairs = [divmod(int(c, 16), 4) for c in TUNING["pairs"]]
    units = [(i, 2 * j + u) for i, j in pairs for u in range(2)]

    light = [n for n in range(35) if len(A_SIDE[n // 5]) == 1]
    heavy = [n for n in range(35) if n not in light]
    x_jobs = [[(light if (knob("x_jobs", n) > 1 and light) or not heavy else heavy).pop(0)
               for _ in range(knob("x_jobs", n))] for n in range(len(units))]
    assert not light and not heavy

    is_outer = lambda n: n.terms and len(wo_parts([n])) == 2 and not any(ch.terms for _, ch in n.terms)
    sources = lambda n: [n] if is_outer(n) or not n.terms else [m for _, ch in n.terms for m in sources(ch)]
    todo = [(n, u) for n in dict.fromkeys(n for r in o_roots for n in sources(r)) if n.terms for u in range(2)]
    sizes, home, sums = [9, 9, 9, 9, 45], {}, []
    for n, unit in enumerate(units):
        arena = (n + 2) // 8
        ready = [(m, u) for m, u in todo if all((i, 2 * j + u) in units[:n + 1] for i, j in leaves(m))]
        sums.append(ready[:knob("sums", n)] if n + 1 < len(units) else ready)
        todo = [key for key in todo if key not in sums[-1]]
        for key in [unit] + sums[-1]:
            home[key] = (arena, sizes[arena])
            sizes[arena] += 1

    def kernel(ax, ak, av, awq, awo, bx, bk, bv, bwq, bwo, out,
               arenas, q_parts, x_buf, xc_buf, wq_buf, wo_buf, kv_buf, y_buf, sem):
        copy = pltpu.make_async_copy
        batch0 = lambda t: t & 4
        head0 = lambda t: (t & 3) * G

        def k_copy(src, t, i, j):
            return copy(src.at[batch0(t) + i, pl.ds(head0(t) + 2 * j, 2)],
                        kv_buf.at[i, j, 0], sem.at[4 * i + j])

        def v_copy(src, t, i, j):
            return copy(src.at[batch0(t) + i, pl.ds(head0(t) + 2 * j, 2)],
                        kv_buf.at[i, j, 1], sem.at[4 * i + j])

        def kv_wait(i, j):
            copy(kv_buf.at[i, j], kv_buf.at[i, j], sem.at[4 * i + j]).wait()

        def wq_copy(src, t, k, j):
            cols = pl.ds(pl.multiple_of((head0(t) + 4 * j) * DH, 512), 512)
            return copy(src.at[pl.ds(256 * k, 256), cols], wq_buf.at[t & 3, k, j], sem.at[16 + 2 * k + j])

        def wo_copy(src, t, k, j):
            rows = pl.ds(pl.multiple_of((head0(t) + 4 * j) * DH, 512), 512)
            return copy(src.at[rows, pl.ds(256 * k, 256)], wo_buf.at[t & 3, k, j], sem.at[20 + 2 * k + j])

        def x_copy(src, t, c=None):
            rows = pl.ds(0, HQ) if c is None else pl.ds(pl.multiple_of(16 * c, 16), 16)
            return copy(src.at[pl.ds(2 * batch0(t), 8), rows], x_buf.at[(t >> 2) & 1, :, rows],
                        sem.at[25 if c is None else 25 + c])

        def y_copy(t, i, k):
            cols = pl.ds(pl.multiple_of((t >> 3) * D + 128 * k, 128), 128)
            return copy(y_buf.at[4 * i + k], out.at[batch0(t) + i, :, cols], sem.at[24])

        def prefetch(make, a_src, b_src, t, mask, *args):
            pl.when((t & (24 | mask)) == 0)(lambda: make(a_src, t, *args).start())
            pl.when((t & (24 | mask)) == 8)(lambda: make(b_src, t, *args).start())

        def combine_x(p, raw, side, rows):
            cache = {}
            vals = [widened(n, lambda b, i, k: x_buf[raw, 2 * b + i, rows, lanes(k)], cache) for n in x_roots[p]]

            def store(q0, q1):
                xc_buf[pl.ds(X_BLOCKS * side + 13 * p + q0, q1 - q0), rows, :] = jnp.stack(
                    [jnp.concatenate(vals[2 * q:2 * q + 2], 1) for q in range(q0, q1)]).astype(BF16)
            return store

        def q_projection(line, t):
            waited, recent = [], {}

            def arrive(g):
                for part in wq_parts(wq_roots[max(4 * g - 2, 0):4 * g + 2]):
                    if part not in waited:
                        waited.append(part)
                        pl.when((t & 4) == 0)(lambda: wq_copy(awq, t, *part).wait())

            arrive(0)
            base, group = X_BLOCKS * ((t >> 2) & 1), t & 3
            for g in range(46):
                members, cache = list(range(max(4 * g - 2, 0), 4 * g + 2)), {}
                leaf = lambda k, h: wq_buf[group, k // 2, h // 4, lanes(k % 2), lanes(h % 4)]
                ws = [evaluate(wq_roots[n], leaf, cache).astype(BF16) for n in members]
                arrive(g + 1)
                if g == 43:
                    pl.when(jnp.logical_and((t & 3) == 1, t < STEPS - 4))(lambda: x_copy(ax, t + 3).wait())
                    kv_wait(*pairs[0])
                xs = [xc_buf[base + 13 * q_order[n][0] + q_order[n][1] // 2, :, lanes(q_order[n][1] % 2)]
                      for n in members]
                t0 = line.now
                for r0, r1 in ((0, HQ),) if g else ((0, 64), (64, HQ)):
                    vals, res = [v[r0:r1] for v in xs], {}
                    if r0 == 0:
                        vals[0] = pltpu.bitcast(line.paced(pltpu.bitcast(vals[0], F32), step=8), BF16)
                    for n, v, w in zip(members, vals, ws):
                        known = {**recent, **res}
                        terms = [(s, known[m] if m in known else line.get(q_parts, m)) for s, m in absorbed.get(n, [])]
                        res[n] = accumulate(None, terms + [(1, jnp.dot(v, w, preferred_element_type=F32))])
                    line.put(t0 + TUNING["q_lag"], q_parts, members[0], r0, list(res.values()))
                recent = res if g else {}

        def out_projection(line, t):
            acc, waited, group = arenas[4], [], t & 3

            def arrive(g):
                for part in wo_parts(wo_roots[2 * g:2 * g + 2]):
                    if part not in waited:
                        waited.append(part)
                        pl.when((t & 4) == 0)(lambda: wo_copy(awo, t, *part).wait())

            def fold(plan, t0, r0, res):
                def old(blk):
                    while r0 == 0 and line.pending.get((id(acc), blk), 0):
                        line.tick()
                    return acc[blk, pl.ds(r0, res[0].shape[0]), :]

                def emit(i, k, val, c0, c1):
                    y_buf[4 * i + k, pl.ds(r0 + 16 * c0, 16 * (c1 - c0)), :] = val[16 * c0:16 * c1]
                    line.ties["y"] = lambda: y_buf[line.ordered(y_buf.shape[0] - 1), pl.ds(0, 16), :]
                    if r0 + 16 * c1 == SQ:
                        pl.when((t & 3) == 3)(lambda: y_copy(t, i, k).start())

                inner = {}
                for (p, r, c), terms, started, complete in plan[0]:
                    blk = 16 + 4 * p + 2 * r + c
                    inner[p, r, c] = accumulate(old(blk) if started else None, [(s, res[n]) for s, n in terms])
                    if not complete:
                        line.put(t0, acc, blk, r0, [inner[p, r, c]])
                for (i, k), terms, started, complete in plan[1]:
                    val = old(4 * i + k)
                    val = accumulate(val if started else jnp.where((t & 3) == 0, 0.0, val),
                                     [(s, inner[key]) for s, key in terms])
                    line.put(t0, acc, 4 * i + k, r0, [val])
                    if complete:
                        line.spread(t0, val.shape[0] // 16, functools.partial(emit, i, k, val.astype(BF16)))

            arrive(0)
            yield
            for g, plan in enumerate(y_plan):
                members, cache = list(range(2 * g, min(2 * g + 2, len(o_order)))), {}
                rows = HQ * len(members)
                leaf = lambda k, j: wo_buf[group, k // 2, j // 2, pl.ds(256 * (j % 2), 256), lanes(k % 2)]
                ws = [evaluate(wo_roots[p], leaf, cache).astype(BF16) for p in members]
                arrive(g + 1)
                cache = {}
                for n in dict.fromkeys(n for p in members for n in sources(o_roots[p])):
                    v = [fetch(line, (n, u) if n.terms else (n.key[0], 2 * n.key[1] + u)) for u in range(2)]
                    cache[n] = jnp.concatenate([v[0] if cache else line.paced(v[0], rows), v[1]], 1)
                xs = [evaluate(o_roots[p], None, cache) for p in members]
                t0 = line.now - rows // 16 + TUNING["y_lag"]
                for r0 in range(0, SQ, rows):
                    fold(plan, t0, r0, [jnp.dot(v[r0:r0 + rows].astype(BF16), w, preferred_element_type=F32)
                                        for v, w in zip(xs, ws)])
                yield

        def fetch(line, key):
            return line.get(arenas[home[key][0]], home[key][1])

        def attention(line, t, projection):
            def background(n):
                def some(store, c0, c1):
                    store(2 * c0, min(2 * c1, 13))
                    line.ties["x"] = lambda: xc_buf[line.zero, pl.ds(0, 16), lanes(0)]

                for job in x_jobs[n]:
                    row = jnp.clip((t & 3) * 40 - 40, 0, HQ - 40) + 8 * (job % 5)
                    store = combine_x(job // 5, ((t + 3) >> 2) & 1, ((t >> 2) + 1) & 1, pl.ds(pl.multiple_of(row, 8), 8))
                    line.spread(line.now + knob("x_lag", n), 7, functools.partial(some, store))

            def scores(n):
                i, h = units[n]
                if n in (3, 5, 7, 9):
                    prefetch(wq_copy, awq, bwq, t + 1, 4, *wq_parts(wq_roots)[n // 2 - 1])
                if n == 11:
                    prefetch(x_copy, ax, bx, t + 4, 3)
                if 12 <= n < 28:
                    pl.when(jnp.logical_and((t & 3) == 0, t > 0))(lambda: y_copy(t - 1, *divmod(n - 12, 4)).wait())
                if n == TUNING["wo_wait"]:
                    next(projection)
                if n % 2 == 0 and n:
                    kv_wait(i, h // 2)
                if n:
                    line.current = arenas[n // 8]
                q = []
                for r in range(2):
                    terms = sorted(q_outs[i, r, h].items(), key=lambda ms: (-ms[1], ms[0]))
                    lead = line.paced(line.get(q_parts, terms[0][0]))
                    rest = [(s, line.get(q_parts, m)) for m, s in terms[1:]]
                    cut = max(len(rest) - knob("q_tail", n), 0)
                    q.append(accumulate(accumulate(None, rest[:cut]), [(terms[0][1], lead)] + rest[cut:]))
                q = (jnp.concatenate(q, 0) * Q_SCALE).astype(BF16)
                s = lax.dot_general(q, kv_buf[i, h // 2, 0, h % 2], (((1,), (1,)), ((), ())), preferred_element_type=F32)
                line.put(line.now - NC + knob("s_lag", n), arenas[n // 8], 4 * (n % 2), 0,
                         [column(s, j) for j in range(4)])

            def first_tile(n, t0):
                ref, blk, got = arenas[n // 8], 4 * (n % 2), []

                def one(c):
                    assert line.pending[id(ref), blk] < NC - c
                    ordered = (line.now + 1) % 2 == line.phase
                    v = ref[line.ordered(blk) if ordered else blk, pl.ds(16 * c, 16), :]
                    if ordered and ref is not line.current:
                        v = jnp.where(line.zero == 0, v, line.marker(16))
                    got.append(v)

                for c in range(NC):
                    line.reads.setdefault(t0 + c - knob("max_lead", n), []).append(lambda c=c: one(c))
                return got

            def values(n, first):
                i, h = units[n]
                ref, blk, probs = arenas[n // 8], 4 * (n % 2), []
                totals = (line.current, 8 if n + 1 < len(units) else 44)
                for c0 in (0, NC // 2):
                    rows = pl.ds(16 * c0, HQ)
                    assert line.pending[id(ref), blk] == 0
                    s = [jnp.concatenate(first[c0:c0 + NC // 2], 0)] + [ref[blk + j, rows, :] for j in range(1, 4)]
                    m = jnp.max(jnp.maximum(jnp.maximum(s[3], s[1]), jnp.maximum(s[2], s[0])), axis=-1, keepdims=True)
                    s = ref[pl.ds(blk, 4), rows, :]
                    e = jnp.exp2(jnp.concatenate([s[j] - m for j in range(4)], 1))
                    line.put(line.now + knob("l_lag", n), *totals, 16 * c0,
                             [(column(e, 0) + column(e, 1)) + (column(e, 2) + column(e, 3))], line.now + NC - 1 - c0)
                    probs.append(jnp.concatenate([line.paced(column(e, 0)), e[:, 128:]], 1))
                o = jnp.dot(jnp.concatenate(probs, 0).astype(BF16), kv_buf[i, h // 2, 1, h % 2], preferred_element_type=F32)
                total = jnp.sum(line.get(*totals), axis=-1, keepdims=True)
                inv = pltpu.reciprocal(total, approx=True)
                o = o * (inv * (2.0 - total * inv))
                both = [evaluate(node, lambda a, j: o if (a, 2 * j + u) == (i, h) else fetch(line, (a, 2 * j + u)), {})
                        for node, u in sums[n]]
                line.put(line.now - NC + knob("o_lag", n), arenas[home[i, h][0]], home[i, h][1], 0, [o] + both)
                if n + 2 < len(units):
                    background(n + 2)
                if n % 2 == 1:
                    prefetch(k_copy, ak, bk, t + 1, 0, i, h // 2)
                    prefetch(v_copy, av, bv, t + 1, 0, i, h // 2)

            line.phase = line.now % 2
            scores(0)
            for n in range(len(units)):
                first = first_tile(n, line.now + NC)
                if n + 1 < len(units):
                    scores(n + 1)
                else:
                    line.current = arenas[4]
                    next(projection)
                values(n, first)
            line.phase = 0

        for c in range(HQ // 16):
            x_copy(ax, 0, c).start()
        for part in wq_parts(wq_roots):
            wq_copy(awq, 0, *part).start()
        for i, j in pairs:
            k_copy(ak, 0, i, j).start()
            v_copy(av, 0, i, j).start()
        for part in wo_parts(wo_roots):
            wo_copy(awo, 0, *part).start()

        for ref in (*arenas, q_parts, y_buf):
            ref[ref.shape[0] - 1, pl.ds(0, 16), :] = jnp.zeros((16, 128), ref.dtype)
        arenas[4][pl.ds(0, 16)] = jnp.zeros((16, SQ, 128), F32)

        def first_operands(c, carry):
            x_copy(ax, 0, c).wait()
            for half in range(2):
                for p in range(7):
                    combine_x(p, 0, 0, pl.ds(pl.multiple_of(16 * c + 8 * half, 8), 8))(0, 13)
            return carry

        lax.fori_loop(0, HQ // 16, first_operands, 0)

        def step(t, carry):
            line = Timeline(t >> 8, q_parts)
            q_projection(line, t)
            projection = out_projection(line, t)
            attention(line, t, projection)
            for _ in projection:
                pass
            for part in wo_parts(wo_roots):
                prefetch(wo_copy, awo, bwo, t + 1, 4, *part)
            while line.events:
                line.tick()
            return carry

        lax.fori_loop(0, STEPS, step, 0)
        for i in range(4):
            for k in range(4):
                y_copy(STEPS - 1, i, k).wait()

    def call(*args):
        args = [a.reshape(2 * B, HQ, D) if n % 5 == 0 else a for n, a in enumerate(args)]
        return pl.pallas_call(
            kernel,
            in_specs=[pl.BlockSpec(memory_space=pl.ANY)] * 10,
            out_specs=pl.BlockSpec(memory_space=pl.ANY),
            out_shape=jax.ShapeDtypeStruct((B, SQ, 2 * D), BF16),
            scratch_shapes=[
                [pltpu.VMEM((n + 1, SQ, 128), F32) for n in sizes],
                pltpu.VMEM((len(q_order) + 2, HQ, 128), F32),
                pltpu.VMEM((2, 8, HQ, D), BF16),
                pltpu.VMEM((2 * X_BLOCKS, HQ, 256), BF16),
                pltpu.VMEM((4, 2, 2, 256, 512), BF16),
                pltpu.VMEM((4, 2, 2, 512, 256), BF16),
                pltpu.VMEM((4, G // 2, 2, 2, SK, DH), BF16),
                pltpu.VMEM((18, SQ, 128), BF16),
                pltpu.SemaphoreType.DMA((32,)),
            ],
            compiler_params=pltpu.CompilerParams(
                vmem_limit_bytes=100 * 1024 * 1024,
                flags={"XLA_TPU_RESCHEDULE_DMA_DONES": True},
                disable_bounds_checks=True,
                disable_semaphore_checks=True,
            ),
        )(*args)
    return call


@jax.jit
def pallas_concat_heads__gqa_block_cached__mha_block_cached__near_ridge_kernel(
    A_x: jax.Array,
    A_k_cache: jax.Array,
    A_v_cache: jax.Array,
    A_wq: jax.Array,
    A_wo: jax.Array,
    B_x: jax.Array,
    B_k_cache: jax.Array,
    B_v_cache: jax.Array,
    B_wq: jax.Array,
    B_wo: jax.Array,
):
    return build()(A_x, A_k_cache, A_v_cache, A_wq, A_wo, B_x, B_k_cache, B_v_cache, B_wq, B_wo)
```
